```python
import os as _os
_os.environ.setdefault("JAX_PLATFORMS", "cpu")
import jax
import jax.numpy as jnp

def _softmax(x, axis=-1):
    return jax.nn.softmax(x, axis=axis)
def _gelu(x):
    return jax.nn.gelu(x, approximate=True)
def _silu(x):
    return jax.nn.silu(x)
def _sigmoid(x):
    return jax.nn.sigmoid(x)
def _layernorm(x, axis=-1, eps=1e-5):
    m = jnp.mean(x, axis=axis, keepdims=True)
    v = jnp.var(x, axis=axis, keepdims=True)
    return (x - m) / jnp.sqrt(v + eps)
def _scatter_add(tgt, idx, src, axis=0):
    return tgt.at[idx].add(src)
def _segment_sum(src, seg, n):
    return jax.ops.segment_sum(src, seg, n)
class _Rng:
    def __init__(self, key):
        self._k = key
    def _next(self):
        self._k, sub = jax.random.split(self._k)
        return sub
    def normal(self, shape):
        return jax.random.normal(self._next(), shape, dtype=jnp.bfloat16)
    def randint(self, lo, hi, shape):
        return jax.random.randint(self._next(), shape, lo, hi, dtype=jnp.int32)
    def uniform(self, shape, lo=0.0, hi=1.0):
        return jax.random.uniform(self._next(), shape, jnp.bfloat16, lo, hi)
    def permutation(self, n):
        return jax.random.permutation(self._next(), n)


kernel_name = 'concat_heads__sliding_block_cached__compressed_kv_cla__decode'

def setup_inputs():
    _rng = _Rng(jax.random.key(int.from_bytes(__import__("os").urandom(4), "little")))
    _w = (lambda a: (lambda t: t.astype(jnp.bfloat16) if jnp.issubdtype(t.dtype, jnp.floating) else t)(jnp.asarray(a)))
    def _A_setup():
        B, Sq, D = 1, 1, 512
        Hq, Hkv, Sk, Dh = 32, 32, 4096, 128
        assert Hq % Hkv == 0, (Hq, Hkv)
        return {
            "x": _w((lambda *s: _rng.normal(s) * 0.8)(B, Sq, D)),
            "k_cache": _w((lambda *s: _rng.normal(s) * 0.8)(B, Hkv, Sk, Dh)),
            "v_cache": _w((lambda *s: _rng.normal(s) * 0.05)(B, Hkv, Sk, Dh)),
            "wq": _w((lambda *s: _rng.normal(s) * 0.8)(D, Hq * Dh) * (D ** -0.5)),
            "wo": _w((lambda *s: _rng.normal(s) * 0.05)(Hq * Dh, D) * ((Hq * Dh) ** -0.5)),
        }
    _A_in = _A_setup()

    def _B_setup():
        B, H, Sq, Sk, D, M = 1, 32, 1, 4096, 128, 512
        Dc = 4 * D
        return {
            "x": _w((lambda *s: _rng.normal(s) * 1.6)(B, Sq, M)),
            "c_kv": _w((lambda *s: _rng.normal(s) * 0.1)(B, Sk, Dc)),
            "w_q": _w((lambda *s: _rng.normal(s) * 1.6)(M, H, D) * (M ** -0.5)),
            "w_uk": _w((lambda *s: _rng.normal(s) * 1.6)(Dc, H, D) * (Dc ** -0.5)),
            "w_uv": _w((lambda *s: _rng.normal(s) * 0.1)(Dc, H, D) * (Dc ** -0.5)),
            "w_o": _w((lambda *s: _rng.normal(s) * 0.1)(H, D, M) * ((H * D) ** -0.5)),
        }
    _B_in = _B_setup()

    return {
        "A_x": _A_in["x"],
        "A_k_cache": _A_in["k_cache"],
        "A_v_cache": _A_in["v_cache"],
        "A_wq": _A_in["wq"],
        "A_wo": _A_in["wo"],
        "B_x": _B_in["x"],
        "B_c_kv": _B_in["c_kv"],
        "B_w_q": _B_in["w_q"],
        "B_w_uk": _B_in["w_uk"],
        "B_w_uv": _B_in["w_uv"],
        "B_w_o": _B_in["w_o"],
    }

def reference(A_x, A_k_cache, A_v_cache, A_wq, A_wo, B_x, B_c_kv, B_w_q, B_w_uk, B_w_uv, B_w_o):
    def _A_ref(x, k_cache, v_cache, wq, wo):
        B, Sq, D = x.shape
        Hq, Dh = 32, 128
        Hkv, Sk = k_cache.shape[1], k_cache.shape[2]
        W = min(4096, max(256, Sk // 4))
        rep = Hq // Hkv
        q = (lambda x, *d: x.transpose(*d))((x @ wq).reshape(B, Sq, Hq, Dh), 0, 2, 1, 3)
        k = jnp.repeat(k_cache[:, :, Sk - W:, :], rep, axis=1)
        v = jnp.repeat(v_cache[:, :, Sk - W:, :], rep, axis=1)
        scores = jnp.einsum("bhqd,bhkd->bhqk", q, k) * (Dh ** -0.5)
        p = _softmax(scores, axis=-1)
        o = jnp.einsum("bhqk,bhkd->bhqd", p, v)
        return (lambda x, *d: x.transpose(*d))(o, 0, 2, 1, 3).reshape(B, Sq, Hq * Dh) @ wo

    def _B_ref(x, c_kv, w_q, w_uk, w_uv, w_o):
        B, Sq, M = x.shape[0], x.shape[1], x.shape[2]
        Sk = c_kv.shape[1]
        H, D = w_q.shape[1], w_q.shape[2]
        q = jnp.einsum("bqm,mhd->bhqd", x, w_q)
        k = jnp.einsum("bkc,chd->bhkd", c_kv, w_uk)
        v = jnp.einsum("bkc,chd->bhkd", c_kv, w_uv)
        scores = jnp.einsum("bhqd,bhkd->bhqk", q, k) * (D ** -0.5)
        off = Sk - Sq
        qi = jnp.arange(Sq)[:, None]
        kj = jnp.arange(Sk)[None, :]
        cmask = kj <= (qi + off)
        scores = jnp.where(cmask[None, None], scores, -1e9)
        p = _softmax(scores, axis=-1)
        ctx = jnp.einsum("bhqk,bhkd->bhqd", p, v)
        return jnp.einsum("bhqd,hdm->bqm", ctx, w_o)

    a = _A_ref(A_x, A_k_cache, A_v_cache, A_wq, A_wo)
    b = _B_ref(B_x, B_c_kv, B_w_q, B_w_uk, B_w_uv, B_w_o)
    return jnp.concatenate([a, b], axis=-1)
```

```python
import functools
import jax
import jax.numpy as jnp
from jax import lax
import jax.experimental.pallas as pl
import jax.experimental.pallas.tpu as pltpu

F32 = jnp.float32
BF16 = jnp.bfloat16
H, DH, DM, DC, SK, WIN = 32, 128, 512, 512, 4096, 1024
NT = (((1,), (1,)), ((), ()))

S_BWQ, S_WUK, S_CKV, S_WUV, S_WQ, S_KV0, S_BWO, S_WO = 0, 1, 2, 3, 4, 5, 9, 10


def _kernel(ax_h, k_h, v_h, wq_h, wo_h, bx_h, c_h, bwq_h, wuk_h, wuv_h, bwo_h, o_ref,
            ax, bx, kb, vb, wqb, wob, cb, bwqb, wukb, wuvb, bwob,
            vr_s, ql_s, sc_s, qa_s, oa_s, ob_s, sems, xsems):

    def slab_copy(src, dst, stage):
        return lambda j: pltpu.make_async_copy(src.at[j], dst.at[j], sems.at[4 * stage + j])

    def kv_copy(g, j):
        src, dst = (k_h, kb) if j < 2 else (v_h, vb)
        h0 = 8 * g + 4 * (j % 2)
        return pltpu.make_async_copy(
            src.at[pl.ds(h0, 4), pl.ds(SK - WIN, WIN)], dst.at[pl.ds(h0, 4)],
            sems.at[4 * (S_KV0 + g) + j])

    cp_bwq = slab_copy(bwq_h, bwqb, S_BWQ)
    cp_wuk = slab_copy(wuk_h, wukb, S_WUK)
    cp_c = slab_copy(c_h, cb, S_CKV)
    cp_wuv = slab_copy(wuv_h, wuvb, S_WUV)
    cp_wq = slab_copy(wq_h, wqb, S_WQ)
    cp_bwo = slab_copy(bwo_h, bwob, S_BWO)
    cp_wo = slab_copy(wo_h, wob, S_WO)
    cp_ax = pltpu.make_async_copy(ax_h, ax, xsems.at[0])
    cp_bx = pltpu.make_async_copy(bx_h, bx, xsems.at[1])

    cp_bwq(0).start()
    cp_bx.start()
    cp_ax.start()
    for j in range(1, 4):
        cp_bwq(j).start()
    for j in range(4):
        cp_wuk(j).start()

    row = lax.broadcasted_iota(jnp.int32, (H, 128), 0)
    lane = lax.broadcasted_iota(jnp.int32, (H, 128), 1)
    diag = (lane & 31) == row
    row8 = lax.broadcasted_iota(jnp.int32, (8, 128), 0)

    def skew(v, sign):
        for bit in range(5):
            sh = (sign * (1 << bit)) % 128
            v = jnp.where(((row >> bit) & 1) == 1, pltpu.roll(v, sh, 1), v)
        return v

    def slab_contract(w_ref, cp, nxt):
        def body(b, acc):
            cp(b).wait()
            nxt(b)
            vr = vr_s[b]
            for s in range(32):
                r = vr if s == 0 else pltpu.roll(vr, 128 - s, 1)
                l = jnp.where(diag, r, 0.0).astype(BF16)
                w = w_ref[b, :, s].reshape(128, 128)
                acc = acc + jnp.dot(l, w, preferred_element_type=F32)
            return acc
        return lax.fori_loop(0, 4, body, jnp.zeros((H, DH), F32))

    cp_bx.wait()
    xb = bx[...].astype(F32)
    for b in range(4):
        vr_s[b] = skew(jnp.broadcast_to(xb[:, 128 * b:128 * (b + 1)], (H, 128)), 1)
    qb = slab_contract(bwqb, cp_bwq, lambda b: cp_c(b).start()).astype(BF16)

    def qlat_body(b, _):
        cp_wuk(b).wait()
        cp_wuv(b).start()
        a = jnp.zeros((H, 128), F32)
        for s in range(32):
            w = wukb[b, :, s].reshape(128, 128)
            r = lax.dot_general(qb, w, NT, preferred_element_type=F32)
            r = jnp.where(diag, r, 0.0)
            a = a + (r if s == 0 else pltpu.roll(r, s, 1))
        ql_s[b] = skew(a, -1)
        return 0
    lax.fori_loop(0, 4, qlat_body, 0)
    ql = jnp.concatenate([ql_s[b] for b in range(4)], axis=1).astype(BF16)

    def score_body(j, m):
        cp_c(j).wait()
        cp_wq(j).start()
        s = lax.dot_general(ql, cb[j], NT, preferred_element_type=F32) * (DH ** -0.5)
        sc_s[j] = s
        for t in range(8):
            m = jnp.maximum(m, s[:, 128 * t:128 * (t + 1)])
        return m
    m = lax.fori_loop(0, 4, score_body, jnp.full((H, 128), -jnp.inf, F32))
    m = jnp.max(m, axis=1, keepdims=True)

    for j in range(4):
        kv_copy(0, j).start()

    def pv_body(j, carry):
        l, acc = carry
        p = jnp.exp(sc_s[j] - m)
        for t in range(8):
            l = l + p[:, 128 * t:128 * (t + 1)]
        acc = acc + jnp.dot(p.astype(BF16), cb[j], preferred_element_type=F32)
        return l, acc
    l, cl = lax.fori_loop(0, 4, pv_body, (jnp.zeros((H, 128), F32), jnp.zeros((H, DC), F32)))
    cl = cl / jnp.sum(l, axis=1, keepdims=True)
    for b in range(4):
        vr_s[b] = skew(cl[:, 128 * b:128 * (b + 1)], 1)

    ctx = slab_contract(wuvb, cp_wuv, lambda b: None)
    for g in range(4):
        ob_s[g] = ctx[8 * g:8 * (g + 1)]

    for j in range(4):
        kv_copy(1, j).start()
    cp_ax.wait()
    xa = ax[...].astype(F32)
    for b in range(4):
        vr_s[b, 0:8] = jnp.broadcast_to(xa[:, 128 * b:128 * (b + 1)], (8, 128))

    def qa_body(j, acc):
        cp_wq(j).wait()
        x8 = vr_s[j, 0:8].astype(BF16)
        r = jnp.dot(x8, wqb[j], preferred_element_type=F32)
        out = []
        for g in range(4):
            a = acc[g]
            for i in range(8):
                h = 8 * g + i
                a = a + jnp.where(row8 == i, r[:, 128 * h:128 * (h + 1)], 0.0)
            out.append(a)
        return tuple(out)
    qa = lax.fori_loop(0, 4, qa_body, tuple(jnp.zeros((8, 128), F32) for _ in range(4)))
    for g in range(4):
        qa_s[g] = qa[g]

    row8w = lax.broadcasted_iota(jnp.int32, (8, WIN), 0)

    def attn_body(g, _):
        q = qa_s[g].astype(BF16)
        s = jnp.zeros((8, WIN), F32)
        for half in range(2):
            kv_copy(g, half).wait()

            @pl.when(g < 2)
            def _():
                kv_copy(g + 2, half).start()

            @pl.when(g == 2)
            def _():
                cp_bwo(half).start()

            @pl.when(g == 3)
            def _():
                cp_wo(half).start()
            for i in range(4 * half, 4 * half + 4):
                r = lax.dot_general(q, kb[8 * g + i], NT, preferred_element_type=F32)
                s = jnp.where(row8w == i, r, s)
        s = s * (DH ** -0.5)
        p = jnp.exp(s - jnp.max(s, axis=1, keepdims=True))
        l = jnp.sum(p, axis=1, keepdims=True)
        p = p.astype(BF16)
        o = jnp.zeros((8, DH), F32)
        for half in range(2):
            kv_copy(g, 2 + half).wait()

            @pl.when(g < 2)
            def _():
                kv_copy(g + 2, 2 + half).start()

            @pl.when(g == 2)
            def _():
                cp_bwo(2 + half).start()

            @pl.when(g == 3)
            def _():
                cp_wo(2 + half).start()
            for i in range(4 * half, 4 * half + 4):
                r = jnp.dot(p, vb[8 * g + i], preferred_element_type=F32)
                o = jnp.where(row8 == i, r, o)
        oa_s[g] = o / l
        return 0
    lax.fori_loop(0, 4, attn_body, 0)

    def out_proj(src, w_ref, cp):
        def body(j, acc):
            o = src[j]
            l = jnp.concatenate([jnp.where(row8 == i, o, 0.0) for i in range(8)], axis=1).astype(BF16)
            cp(j).wait()
            return acc + jnp.dot(l, w_ref[j], preferred_element_type=F32)
        acc = lax.fori_loop(0, 4, body, jnp.zeros((8, DM), F32))
        return jnp.sum(acc, axis=0, keepdims=True)

    o_ref[:, DM:] = out_proj(ob_s, bwob, cp_bwo).astype(o_ref.dtype)
    o_ref[:, :DM] = out_proj(oa_s, wob, cp_wo).astype(o_ref.dtype)


@jax.jit
def pallas_concat_heads__sliding_block_cached__compressed_kv_cla__decode_kernel(A_x, A_k_cache, A_v_cache, A_wq, A_wo, B_x, B_c_kv, B_w_q, B_w_uk, B_w_uv, B_w_o):
    hbm = pl.BlockSpec(memory_space=pltpu.MemorySpace.HBM)
    slab = (4, 4, 32, H, DH)
    out = pl.pallas_call(
        _kernel,
        in_specs=[hbm] * 11,
        out_specs=pl.BlockSpec(memory_space=pltpu.MemorySpace.VMEM),
        out_shape=jax.ShapeDtypeStruct((1, 2 * DM), A_x.dtype),
        scratch_shapes=[
            pltpu.VMEM((1, DM), BF16), pltpu.VMEM((1, DM), BF16),
            pltpu.VMEM((H, WIN, DH), BF16), pltpu.VMEM((H, WIN, DH), BF16),
            pltpu.VMEM((4, 128, H * DH), BF16), pltpu.VMEM((4, 1024, DM), BF16),
            pltpu.VMEM((4, 1024, DC), BF16),
            pltpu.VMEM(slab, BF16), pltpu.VMEM(slab, BF16), pltpu.VMEM(slab, BF16),
            pltpu.VMEM((4, 1024, DM), BF16),
            pltpu.VMEM((4, H, 128), F32), pltpu.VMEM((4, H, 128), F32),
            pltpu.VMEM((4, H, 1024), F32),
            pltpu.VMEM((4, 8, 128), F32), pltpu.VMEM((4, 8, 128), F32), pltpu.VMEM((4, 8, 128), F32),
            pltpu.SemaphoreType.DMA((44,)), pltpu.SemaphoreType.DMA((2,)),
        ],
        compiler_params=pltpu.CompilerParams(vmem_limit_bytes=100 * 1024 * 1024),
    )(
        A_x.reshape(1, DM), A_k_cache.reshape(H, SK, DH), A_v_cache.reshape(H, SK, DH),
        A_wq.reshape(4, 128, H * DH), A_wo.reshape(4, 1024, DM),
        B_x.reshape(1, DM), B_c_kv.reshape(4, 1024, DC),
        B_w_q.reshape(slab), B_w_uk.reshape(slab), B_w_uv.reshape(slab),
        B_w_o.reshape(4, 1024, DM),
    )
    return out.reshape(1, 1, 2 * DM)
```

```python
import functools
import jax
import jax.numpy as jnp
from jax import lax
import jax.experimental.pallas as pl
import jax.experimental.pallas.tpu as pltpu

F32 = jnp.float32
BF16 = jnp.bfloat16
H, DH, DM, DC, SK, WIN = 32, 128, 512, 512, 4096, 1024
NT = (((1,), (1,)), ((), ()))
CFG = dict(subs=(0, 8, 16, 24, 28, 30, 31, 32), la=10, strided_slab=False, compute=True)


def _mul(i, n):
    return i * n if isinstance(i, int) else pl.multiple_of(i * n, n)


def _divmod(j, n):
    return divmod(j, n) if isinstance(j, int) else (lax.div(j, n), lax.rem(j, n))


def _kernel(cfg, ax_h, k_h, v_h, wq_h, wo_h, bx_h, c_h, bwq_h, wuk_h, wuv_h, bwo_h, o_h,
            ax, bx, kb, vb, wqb, cb, bwqb, wukb, wuvb, wob,
            vr_s, ql_s, sc_s, qa_s, pa_s, la_s, lo_s, lt_s, out_v, osem):
    subs = cfg['subs']
    compute = cfg['compute']

    la = cfg['la']

    def streamed(tsems):
        def slab_piece(src, dst, sem, u, j):
            if cfg['strided_slab']:
                return pltpu.make_async_copy(src.at[u, :, j], dst.at[u, :, j], sem)
            i, s = _divmod(j, 8)
            idx = (u, i, pl.ds(_mul(s, 4), 4))
            return pltpu.make_async_copy(src.at[idx], dst.at[idx], sem)

        def row_piece(src, dst, sem, u, ud, j):
            r = pl.ds(_mul(j, 32), 32)
            return pltpu.make_async_copy(src.at[u, r], dst.at[ud, r], sem)

        def wq_piece(sem, u, j):
            t, half = _divmod(j, 2)
            idx = (u, pl.ds(_mul(t, 8), 8), pl.ds(_mul(half, 2048), 2048))
            return pltpu.make_async_copy(wq_h.at[idx], wqb.at[idx], sem)

        def kv_piece(src, dst, sem, u, j):
            t, g = _divmod(j, 4)
            h = 8 * g + u
            return pltpu.make_async_copy(
                src.at[h, pl.ds(SK - WIN + _mul(t, 128), 128)], dst.at[h, pl.ds(_mul(t, 128), 128)], sem)

        def round_copies(sems, phase, j):
            if phase == 0:
                return [c for u in range(4) for c in (
                    slab_piece(bwq_h, bwqb, sems.at[0], u, j), slab_piece(wuk_h, wukb, sems.at[1], u, j))]
            if phase == 1:
                return [c for u in range(4) for c in (
                    row_piece(c_h, cb, sems.at[2], u, u, j), wq_piece(sems.at[3], u, j))]
            if phase == 2:
                return [c for u in range(4) for c in (
                    kv_piece(k_h, kb, sems.at[4], 2 * u, j), slab_piece(wuv_h, wuvb, sems.at[5], u, j),
                    kv_piece(k_h, kb, sems.at[4], 2 * u + 1, j))]
            if phase == 3:
                return [kv_piece(v_h, vb, sems.at[6], u, j) for u in range(8)]
            if isinstance(j, int):
                si = max(i for i in range(len(subs) - 1) if subs[i] <= j)
            else:
                si = sum((j >= b).astype(jnp.int32) for b in subs[1:-1])
            return [c for u in range(4) for c in (
                row_piece(bwo_h, wob, tsems.at[si], u, u, j), row_piece(wo_h, wob, tsems.at[si], u, 4 + u, j))]

        def start_round(sems, phase, j):
            for n, c in enumerate(round_copies(sems, phase, j)):
                c.start(priority=n % 2)

        def issue(sems, phase, j0, j1):
            if j1 - j0 <= 2:
                for j in range(j0, j1):
                    start_round(sems, phase, j)
            else:
                pl.loop(j0, j1)(lambda j: start_round(sems, phase, j))

        def hook(sems, phase, j0, per):
            def f(it):
                for r in range(per):
                    start_round(sems, phase, j0 + it * per + r)
            return f

        def wait_all(buf, sem):
            pltpu.make_async_copy(buf, buf, sem).wait()

        def body(sems, xsems):
            cp_ax = pltpu.make_async_copy(ax_h, ax, xsems.at[0])
            cp_bx = pltpu.make_async_copy(bx_h, bx, xsems.at[1])
            start_round(sems, 0, 0)
            cp_bx.start()
            cp_ax.start()
            issue(sems, 0, 1, 32)
            issue(sems, 1, 0, la)

            row = lax.broadcasted_iota(jnp.int32, (H, 128), 0)
            lane = lax.broadcasted_iota(jnp.int32, (H, 128), 1)
            diag = (lane & 31) == row
            row8 = lax.broadcasted_iota(jnp.int32, (8, 128), 0)

            def skew(v, sign):
                for bit in range(5):
                    sh = (sign * (1 << bit)) % 128
                    v = jnp.where(((row >> bit) & 1) == 1, pltpu.roll(v, sh, 1), v)
                return v

            def slab_contract(w_ref, nxt):
                def step(b, acc):
                    nxt(b)
                    if not compute:
                        return acc
                    vr = vr_s[b]
                    for s in range(32):
                        r = vr if s == 0 else pltpu.roll(vr, 128 - s, 1)
                        l = jnp.where(diag, r, 0.0).astype(BF16)
                        w = w_ref[b, :, s].reshape(128, 128)
                        acc = acc + jnp.dot(l, w, preferred_element_type=F32)
                    return acc
                return lax.fori_loop(0, 4, step, jnp.zeros((H, DH), F32))

            def flat_heads(o):
                return jnp.concatenate(
                    [jnp.broadcast_to(o[i:i + 1], (8, DH)) for i in range(8)], axis=1)

            cp_bx.wait()
            xb = bx[...].astype(F32)
            for b in range(4):
                vr_s[b] = skew(jnp.broadcast_to(xb[:, 128 * b:128 * (b + 1)], (H, 128)), 1)
            wait_all(bwqb, sems.at[0])
            qb = slab_contract(bwqb, hook(sems, 1, la, 2)).astype(BF16)

            wait_all(wukb, sems.at[1])
            nxt = hook(sems, 1, la + 8, 2)

            @pl.loop(0, 4)
            def _(b):
                nxt(b)
                if not compute:
                    return
                a = jnp.zeros((H, 128), F32)
                for s in range(32):
                    w = wukb[b, :, s].reshape(128, 128)
                    r = lax.dot_general(qb, w, NT, preferred_element_type=F32)
                    r = jnp.where(diag, r, 0.0)
                    a = a + (r if s == 0 else pltpu.roll(r, s, 1))
                ql_s[b] = skew(a, -1)
            issue(sems, 1, la + 16, 32)
            la2 = (8 * la + 11) // 12
            issue(sems, 2, 0, la2)
            ql = jnp.concatenate([ql_s[b] for b in range(4)], axis=1).astype(BF16)

            wait_all(cb, sems.at[2])
            nxt1 = hook(sems, 2, la2, 1)

            def score_step(j, m):
                nxt1(j)
                if not compute:
                    return m
                s = lax.dot_general(ql, cb[j], NT, preferred_element_type=F32) * (DH ** -0.5)
                sc_s[j] = s
                for t in range(8):
                    m = jnp.maximum(m, s[:, 128 * t:128 * (t + 1)])
                return m
            m = lax.fori_loop(0, 4, score_step, jnp.full((H, 128), -jnp.inf, F32))
            m = jnp.max(m, axis=1, keepdims=True)
            nxt2 = hook(sems, 2, la2 + 4, 1)

            def pv_step(j, carry):
                nxt2(j)
                if not compute:
                    return carry
                l, acc = carry
                p = jnp.exp(sc_s[j] - m)
                for t in range(8):
                    l = l + p[:, 128 * t:128 * (t + 1)]
                acc = acc + jnp.dot(p.astype(BF16), cb[j], preferred_element_type=F32)
                return l, acc
            l, cl = lax.fori_loop(0, 4, pv_step, (jnp.zeros((H, 128), F32), jnp.zeros((H, DC), F32)))
            cl = cl / jnp.sum(l, axis=1, keepdims=True)
            for b in range(4):
                vr_s[b] = skew(cl[:, 128 * b:128 * (b + 1)], 1)

            cp_ax.wait()
            xa = ax[...].astype(F32)
            for b in range(4):
                qa_s[b] = jnp.broadcast_to(xa[:, 128 * b:128 * (b + 1)], (8, 128))
            wait_all(wqb, sems.at[3])
            nxt3 = hook(sems, 2, la2 + 8, 1)

            def qa_step(j, acc):
                nxt3(j)
                if not compute:
                    return acc
                r = jnp.dot(qa_s[j].astype(BF16), wqb[j], preferred_element_type=F32)
                out = []
                for g in range(4):
                    a = acc[g]
                    for i in range(8):
                        h = 8 * g + i
                        a = a + jnp.where(row8 == i, r[:, 128 * h:128 * (h + 1)], 0.0)
                    out.append(a)
                return tuple(out)
            qa = lax.fori_loop(0, 4, qa_step, tuple(jnp.zeros((8, 128), F32) for _ in range(4)))
            for g in range(4):
                qa_s[g] = qa[g]
            issue(sems, 2, la2 + 12, 32)
            issue(sems, 3, 0, la)

            wait_all(wuvb, sems.at[5])
            ctx = slab_contract(wuvb, hook(sems, 3, la, 2))
            for g in range(4):
                lo_s[g] = flat_heads(ctx[8 * g:8 * (g + 1)])

            wait_all(kb, sems.at[4])
            per = min(3, (32 - la - 8) // 4)
            nxt4 = hook(sems, 3, la + 8, per)
            row8w = lax.broadcasted_iota(jnp.int32, (8, WIN), 0)

            @pl.loop(0, 4)
            def _(g):
                nxt4(g)
                if not compute:
                    return
                q = qa_s[g].astype(BF16)
                s = jnp.zeros((8, WIN), F32)
                for i in range(8):
                    r = lax.dot_general(q, kb[8 * g + i], NT, preferred_element_type=F32)
                    s = jnp.where(row8w == i, r, s)
                s = s * (DH ** -0.5)
                p = jnp.exp(s - jnp.max(s, axis=1, keepdims=True))
                pa_s[g] = p
                la_s[g] = jnp.broadcast_to(jnp.sum(p, axis=1, keepdims=True), (8, 128))
            issue(sems, 3, la + 8 + 4 * per, 32)
            issue(sems, 4, 0, la)

            wait_all(vb, sems.at[6])
            nxt5 = hook(sems, 4, la, 3)

            @pl.loop(0, 4)
            def _(g):
                nxt5(g)
                if not compute:
                    return
                p = pa_s[g].astype(BF16)
                o = jnp.zeros((8, DH), F32)
                for i in range(8):
                    r = jnp.dot(p, vb[8 * g + i], preferred_element_type=F32)
                    o = jnp.where(row8 == i, r, o)
                lo_s[4 + g] = flat_heads(o / la_s[g])

        pl.run_scoped(body, pltpu.SemaphoreType.DMA((7,)), pltpu.SemaphoreType.DMA((2,)))

        acc = [jnp.zeros((8, DM), F32), jnp.zeros((8, DM), F32)]
        issued = min(32, la + 12)
        for si in range(len(subs) - 1):
            r0, r1 = 32 * subs[si], 32 * subs[si + 1]
            upto = min(32, subs[si + 1] + la + 6)
            if upto > issued:
                issue(None, 4, issued, upto)
                issued = upto
            gather = (r1 - r0) % 128 != 0
            if gather and compute:
                lhs = [jnp.concatenate([lo_s[4 * p + u][:, r0:r1] for u in range(4)], axis=1).astype(BF16)
                       for p in range(2)]
            wait_all(wob.at[:, pl.ds(r0, r1 - r0)], tsems.at[si])
            if not compute:
                continue
            for p in range(2):
                if gather:
                    w = wob[4 * p:4 * p + 4, r0:r1].reshape(4 * (r1 - r0), DM)
                    acc[p] = acc[p] + jnp.dot(lhs[p], w, preferred_element_type=F32)
                else:
                    for u in range(4 * p, 4 * p + 4):
                        acc[p] = acc[p] + jnp.dot(
                            lo_s[u, :, r0:r1].astype(BF16), wob[u, r0:r1], preferred_element_type=F32)
        out_v[:, :DM] = acc[1][0:1].astype(out_v.dtype)
        out_v[:, DM:] = acc[0][0:1].astype(out_v.dtype)
        cp_out.start()

    cp_out = pltpu.make_async_copy(out_v, o_h, osem)
    pl.run_scoped(streamed, pltpu.SemaphoreType.DMA((len(subs) - 1,)))
    cp_out.wait()


def make(**over):
    cfg = dict(CFG, **over)

    def kernel(A_x, A_k_cache, A_v_cache, A_wq, A_wo, B_x, B_c_kv, B_w_q, B_w_uk, B_w_uv, B_w_o):
        hbm = pl.BlockSpec(memory_space=pltpu.MemorySpace.HBM)
        slab = (4, 4, 32, H, DH)
        out = pl.pallas_call(
            functools.partial(_kernel, cfg),
            in_specs=[hbm] * 11,
            out_specs=hbm,
            out_shape=jax.ShapeDtypeStruct((1, 2 * DM), A_x.dtype),
            scratch_shapes=[
                pltpu.VMEM((1, DM), BF16), pltpu.VMEM((1, DM), BF16),
                pltpu.VMEM((H, WIN, DH), BF16), pltpu.VMEM((H, WIN, DH), BF16),
                pltpu.VMEM((4, 128, H * DH), BF16), pltpu.VMEM((4, 1024, DC), BF16),
                pltpu.VMEM(slab, BF16), pltpu.VMEM(slab, BF16), pltpu.VMEM(slab, BF16),
                pltpu.VMEM((8, 1024, DM), BF16),
                pltpu.VMEM((4, H, 128), F32), pltpu.VMEM((4, H, 128), F32),
                pltpu.VMEM((4, H, 1024), F32),
                pltpu.VMEM((4, 8, 128), F32), pltpu.VMEM((4, 8, WIN), F32), pltpu.VMEM((4, 8, 128), F32),
                pltpu.VMEM((8, 8, 1024), F32), pltpu.VMEM((8, 128), F32),
                pltpu.VMEM((1, 2 * DM), A_x.dtype), pltpu.SemaphoreType.DMA(()),
            ],
            compiler_params=pltpu.CompilerParams(vmem_limit_bytes=100 * 1024 * 1024),
        )(
            A_x.reshape(1, DM), A_k_cache.reshape(H, SK, DH), A_v_cache.reshape(H, SK, DH),
            A_wq.reshape(4, 128, H * DH), A_wo.reshape(4, 1024, DM),
            B_x.reshape(1, DM), B_c_kv.reshape(4, 1024, DC),
            B_w_q.reshape(slab), B_w_uk.reshape(slab), B_w_uv.reshape(slab),
            B_w_o.reshape(4, 1024, DM),
        )
        return out.reshape(1, 1, 2 * DM)
    return kernel


pallas_concat_heads__sliding_block_cached__compressed_kv_cla__decode_kernel = jax.jit(make())
```

```python
import functools

import jax
import jax.numpy as jnp
from jax import lax
import jax.experimental.pallas as pl
import jax.experimental.pallas.tpu as pltpu

F32 = jnp.float32
BF16 = jnp.bfloat16
H, DH, DM, DC, SK, WIN = 32, 128, 512, 512, 4096, 1024
NT = (((1,), (1,)), ((), ()))

CFG = dict(ahead=10, per=(1, 4, 2, 2, 1, 1, 3, 2), a_cuts=(0, 8, 16, 24, 28, 30), lead=24,
           b_cuts=(0, 8, 16, 24, 32), lag=0, bshift=12, hoist=32, vsplit=3, compute=True, dma=True)


def _mul(i, n):
    return i * n if isinstance(i, int) else pl.multiple_of(i * n, n)


def _divmod(j, n):
    return divmod(j, n) if isinstance(j, int) else (lax.div(j, n), lax.rem(j, n))


def _cut(cuts, j):
    if isinstance(j, int):
        return sum(j >= c for c in cuts[1:-1])
    return sum((j >= c).astype(jnp.int32) for c in cuts[1:-1])


def _kernel(cfg, ax_h, k_h, v_h, wq_h, wo_h, bx_h, c_h, bwq_h, wuk_h, wuv_h, bwo_h, out_h,
            ax, bx, kb, vb, wqb, wob, cb, bwqb, wukb, wuvb, bwob,
            skew_s, ql_s, sb_s, qa_s, pa_s, la_s, oa_s, ob_s, out_v, out_sem):
    ahead, a_cuts, b_cuts, lag = cfg['ahead'], cfg['a_cuts'], cfg['b_cuts'], cfg['lag']
    compute = cfg['compute']
    copy = pltpu.make_async_copy

    def start_all(copies, lead=0):
        if cfg['dma']:
            for n, c in enumerate(copies):
                c.start(priority=1 if n < lead else n % 2)

    def wait_filled(buf, sem):
        if cfg['dma']:
            copy(buf, buf, sem).wait()

    def slab_piece(src, dst, sem, u, j):
        i, s = _divmod(j, 8)
        idx = (u, i, pl.ds(_mul(s, 4), 4))
        return copy(src.at[idx], dst.at[idx], sem)

    def row_piece(src, dst, sem, u, j):
        idx = (u, pl.ds(_mul(j, 32), 32))
        return copy(src.at[idx], dst.at[idx], sem)

    def wq_piece(sem, u, j):
        t, half = _divmod(j, 2)
        idx = (u, pl.ds(_mul(t, 8), 8), pl.ds(_mul(half, 2048), 2048))
        return copy(wq_h.at[idx], wqb.at[idx], sem)

    def cache_round(src, dst, sem, j):
        t, g = _divmod(j, 4)
        r = _mul(t, 128)
        return [copy(src.at[8 * g + u, pl.ds(SK - WIN + r, 128)], dst.at[8 * g + u, pl.ds(r, 128)], sem)
                for u in range(8)]

    def project(asems, bsems):
        def out_round(j):
            b = lambda: [row_piece(bwo_h, bwob, bsems.at[_cut(b_cuts, j)], u, j) for u in range(4)]
            def a_sem(u):
                if isinstance(j, int) and j - lag >= a_cuts[-1]:
                    return asems.at[len(a_cuts) - 1 + (u >= cfg['vsplit'])]
                return asems.at[_cut(a_cuts, j - lag)]
            a = lambda: [row_piece(wo_h, wob, a_sem(u), u, j - lag) for u in range(4)]
            if isinstance(j, int) and (j < lag or j >= 32):
                return b() if j < lag else a()
            return [c for pair in zip(b(), a()) for c in pair]

        pos = [0]
        end = 64 + 32 + lag

        def stream(sems, j, lo, hi):
            parts = ((0, 32, lambda i: cache_round(k_h, kb, sems.at[5], i)),
                     (32, 64, lambda i: cache_round(v_h, vb, sems.at[6], i)),
                     (64, end, out_round))
            for a, b, fn in parts:
                if a <= lo and hi < b:
                    start_all(fn(j - a))
                elif lo < b and a <= hi:
                    pl.when((j >= a) & (j < b))(lambda: start_all(fn(j - a)))

        def issue(sems, upto):
            upto = min(upto, end)
            while pos[0] < upto:
                lo = pos[0]
                hi = min(upto, (lo // 32 + 1) * 32)
                if lo < 64 and hi - lo > 2:
                    pl.loop(lo, hi)(lambda j: stream(sems, j, lo, hi - 1))
                else:
                    for j in range(lo, hi):
                        stream(sems, j, j, j)
                pos[0] = hi

        def hook(sems, per):
            base = pos[0]
            stop = 64 if base < 64 + lag else 96
            pos[0] = max(base, min(base + 4 * per, stop))

            def feed(step, part, n):
                for r in range(per):
                    lo, hi = base + r, base + 3 * per + r
                    if r * n // per != part or lo >= stop:
                        continue
                    j = base + step * per + r
                    if hi < stop:
                        stream(sems, j, lo, hi)
                    else:
                        pl.when(j < stop)(functools.partial(stream, sems, j, lo, stop - 1))
            return feed

        def attend(sems):
            def weights_round(j):
                return [c for u in range(4) for c in (
                    slab_piece(bwq_h, bwqb, sems.at[0], u, j), slab_piece(wuk_h, wukb, sems.at[1], u, j),
                    row_piece(c_h, cb, sems.at[2], u, j), wq_piece(sems.at[3], u, j),
                    slab_piece(wuv_h, wuvb, sems.at[4], u, j))]

            start_all(weights_round(0) + weights_round(1), cfg['lead'])
            cp_ax = copy(ax_h, ax, sems.at[7])
            cp_bx = copy(bx_h, bx, sems.at[8])
            cp_ax.start()
            cp_bx.start()
            pl.loop(2, 32)(lambda j: start_all(weights_round(j)))
            issue(sems, ahead)

            row = lax.broadcasted_iota(jnp.int32, (H, 128), 0)
            lane = lax.broadcasted_iota(jnp.int32, (H, 128), 1)
            diag = (lane & (H - 1)) == row
            row8 = lax.broadcasted_iota(jnp.int32, (8, 128), 0)

            def skew(v, sign):
                for bit in range(5):
                    v = jnp.where(((row >> bit) & 1) == 1, pltpu.roll(v, (sign * (1 << bit)) % 128, 1), v)
                return v

            def slab_contract(w_ref, feed):
                def step(b, acc):
                    vs = skew_s[b]
                    for s in range(32):
                        feed(b, s, 32)
                        if compute:
                            lhs = jnp.where(diag, pltpu.roll(vs, 128 - s, 1) if s else vs, 0.0).astype(BF16)
                            acc = acc + jnp.dot(lhs, w_ref[b, :, s].reshape(128, DH), preferred_element_type=F32)
                    return acc
                return lax.fori_loop(0, 4, step, jnp.zeros((H, DH), F32))

            def flat_heads(o):
                return jnp.concatenate([jnp.broadcast_to(o[i:i + 1], (8, DH)) for i in range(8)], axis=1)

            cp_ax.wait()
            cp_bx.wait()
            xa = ax[...].astype(F32)
            xb = bx[...].astype(F32)
            for b in range(4):
                skew_s[b] = skew(jnp.broadcast_to(xb[:, 128 * b:128 * (b + 1)], (H, 128)), 1)
                qa_s[b] = jnp.broadcast_to(xa[:, 128 * b:128 * (b + 1)], (8, 128))

            wait_filled(bwqb, sems.at[0])
            qb = slab_contract(bwqb, hook(sems, cfg['per'][0])).astype(BF16)

            wait_filled(wukb, sems.at[1])
            feed_ql = hook(sems, cfg['per'][1])

            @pl.loop(0, 4)
            def _(b):
                acc = jnp.zeros((H, 128), F32)
                for s in range(32):
                    feed_ql(b, s, 32)
                    if compute:
                        r = lax.dot_general(qb, wukb[b, :, s].reshape(128, DH), NT, preferred_element_type=F32)
                        r = jnp.where(diag, r, 0.0)
                        acc = acc + (pltpu.roll(r, s, 1) if s else r)
                ql_s[b] = skew(acc, -1)
            ql = jnp.concatenate([ql_s[b] for b in range(4)], axis=1).astype(BF16)

            wait_filled(cb, sems.at[2])
            feed_sb = hook(sems, cfg['per'][2])

            def score_step(j, m):
                for t in range(2):
                    feed_sb(j, t, 2)
                    if compute:
                        s = lax.dot_general(ql, cb[j, 512 * t:512 * (t + 1)], NT,
                                            preferred_element_type=F32) * (DH ** -0.5)
                        sb_s[j, :, 512 * t:512 * (t + 1)] = s
                        for i in range(4):
                            m = jnp.maximum(m, s[:, 128 * i:128 * (i + 1)])
                return m
            m = lax.fori_loop(0, 4, score_step, jnp.full((H, 128), -jnp.inf, F32))
            m = jnp.max(m, axis=1, keepdims=True)
            feed_pb = hook(sems, cfg['per'][3])

            def context_step(j, carry):
                l, acc = carry
                for t in range(2):
                    feed_pb(j, t, 2)
                    if compute:
                        p = jnp.exp(sb_s[j, :, 512 * t:512 * (t + 1)] - m)
                        for i in range(4):
                            l = l + p[:, 128 * i:128 * (i + 1)]
                        acc = acc + jnp.dot(p.astype(BF16), cb[j, 512 * t:512 * (t + 1)],
                                            preferred_element_type=F32)
                return l, acc
            l, cl = lax.fori_loop(0, 4, context_step, (jnp.zeros((H, 128), F32), jnp.zeros((H, DC), F32)))
            cl = cl / jnp.sum(l, axis=1, keepdims=True)
            for b in range(4):
                skew_s[b] = skew(cl[:, 128 * b:128 * (b + 1)], 1)

            wait_filled(wqb, sems.at[3])
            feed_qa = hook(sems, cfg['per'][4])

            def qa_step(j, acc):
                x8 = qa_s[j].astype(BF16)
                new = []
                for g in range(4):
                    feed_qa(j, g, 4)
                    a = acc[g]
                    if compute:
                        r = jnp.dot(x8, wqb[j, :, 1024 * g:1024 * (g + 1)], preferred_element_type=F32)
                        for i in range(8):
                            a = a + jnp.where(row8 == i, r[:, 128 * i:128 * (i + 1)], 0.0)
                    new.append(a)
                return tuple(new)
            qa = lax.fori_loop(0, 4, qa_step, tuple(jnp.zeros((8, DH), F32) for _ in range(4)))
            for g in range(4):
                qa_s[g] = qa[g]

            wait_filled(wuvb, sems.at[4])
            ctx = slab_contract(wuvb, hook(sems, cfg['per'][5]))
            for g in range(4):
                ob_s[g] = flat_heads(ctx[8 * g:8 * (g + 1)])

            issue(sems, 32 + ahead)
            wait_filled(kb, sems.at[5])
            feed_sa = hook(sems, cfg['per'][6])
            row8w = lax.broadcasted_iota(jnp.int32, (8, WIN), 0)

            @pl.loop(0, 4)
            def _(g):
                q = qa_s[g].astype(BF16)
                s = jnp.zeros((8, WIN), F32)
                for i in range(8):
                    feed_sa(g, i, 8)
                    if compute:
                        r = lax.dot_general(q, kb[8 * g + i], NT, preferred_element_type=F32)
                        s = jnp.where(row8w == i, r, s)
                s = s * (DH ** -0.5)
                p = jnp.exp(s - jnp.max(s, axis=1, keepdims=True))
                pa_s[g] = p
                la_s[g] = jnp.broadcast_to(jnp.sum(p, axis=1, keepdims=True), (8, DH))

            issue(sems, 64 + ahead)
            wait_filled(vb, sems.at[6])
            feed_pa = hook(sems, cfg['per'][7])

            @pl.loop(0, 4)
            def _(g):
                p = pa_s[g].astype(BF16)
                o = jnp.zeros((8, DH), F32)
                for i in range(8):
                    feed_pa(g, i, 8)
                    if compute:
                        r = jnp.dot(p, vb[8 * g + i], preferred_element_type=F32)
                        o = jnp.where(row8 == i, r, o)
                oa_s[g] = flat_heads(o / la_s[g])

        pl.run_scoped(attend, pltpu.SemaphoreType.DMA((9,)))

        work = sorted([(b_cuts[i + 1] - cfg['bshift'], 0, i) for i in range(len(b_cuts) - 1)] +
                      [(a_cuts[i + 1] + lag, 1, i) for i in range(len(a_cuts) - 1)])

        def left(o_s, cuts, i):
            return jnp.concatenate([o_s[u, :, 32 * cuts[i]:32 * cuts[i + 1]] for u in range(4)], axis=1).astype(BF16)
        hoisted = {i: left(oa_s, a_cuts, i) for i in range(len(a_cuts) - 1) if a_cuts[i] >= cfg['hoist']}
        acc = [jnp.zeros((8, DM), F32), jnp.zeros((8, DM), F32)]
        if a_cuts[-1] < 32:
            cols = [jnp.broadcast_to(oa_s[u, 0:1, 896:], (128, 128)).T[32 * a_cuts[-1] - 896:] for u in range(4)]
        for last_round, is_a, i in work:
            o_s, w, sems, cuts = (oa_s, wob, asems, a_cuts) if is_a else (ob_s, bwob, bsems, b_cuts)
            r0, r1 = 32 * cuts[i], 32 * cuts[i + 1]
            issue(None, 64 + cuts[i + 1] + ahead)
            lhs = hoisted[i] if is_a and i in hoisted else left(o_s, cuts, i)
            wait_filled(w.at[:, pl.ds(r0, r1 - r0)], sems.at[i])
            if cfg.get('oc', lambda is_a, i: compute)(is_a, i):
                acc[is_a] = acc[is_a] + jnp.dot(lhs, w[:, r0:r1].reshape(4 * (r1 - r0), DM),
                                                preferred_element_type=F32)
            if r1 == 1024:
                c0 = 0 if is_a else DM
                out_v[:, c0:c0 + DM] = acc[is_a][0:1].astype(out_v.dtype)
        if a_cuts[-1] < 32:
            r0 = 32 * a_cuts[-1]
            part = jnp.zeros((8, DM), F32)
            for i, (u0, u1) in enumerate(((0, cfg['vsplit']), (cfg['vsplit'], 4))):
                wait_filled(wob.at[pl.ds(u0, u1 - u0), pl.ds(r0, 1024 - r0)], asems.at[len(a_cuts) - 1 + i])
                for u in range(u0, u1):
                    w = wob[u, r0:].astype(F32)
                    for k in range(0, 1024 - r0, 8):
                        part = part + w[k:k + 8] * jnp.concatenate([cols[u][k:k + 8]] * 4, axis=1)
            out_v[:, :DM] = (acc[1][0:1] + jnp.sum(part, axis=0, keepdims=True)).astype(out_v.dtype)
        cp_out.start()

    cp_out = copy(out_v, out_h, out_sem)
    pl.run_scoped(project, pltpu.SemaphoreType.DMA((len(a_cuts) - 1 + 2 * (a_cuts[-1] < 32),)),
                  pltpu.SemaphoreType.DMA((len(b_cuts) - 1,)))
    cp_out.wait()


def make(**over):
    cfg = dict(CFG, **over)

    def kernel(A_x, A_k_cache, A_v_cache, A_wq, A_wo, B_x, B_c_kv, B_w_q, B_w_uk, B_w_uv, B_w_o):
        hbm = pl.BlockSpec(memory_space=pltpu.MemorySpace.HBM)
        slab, rows, cache = (4, 4, 32, H, DH), (4, 1024, DM), (H, WIN, DH)
        out = pl.pallas_call(
            functools.partial(_kernel, cfg),
            in_specs=[hbm] * 11,
            out_specs=hbm,
            out_shape=jax.ShapeDtypeStruct((1, 2 * DM), A_x.dtype),
            scratch_shapes=[
                pltpu.VMEM((1, DM), BF16), pltpu.VMEM((1, DM), BF16),
                pltpu.VMEM(cache, BF16), pltpu.VMEM(cache, BF16),
                pltpu.VMEM((4, 128, H * DH), BF16), pltpu.VMEM(rows, BF16), pltpu.VMEM(rows, BF16),
                pltpu.VMEM(slab, BF16), pltpu.VMEM(slab, BF16), pltpu.VMEM(slab, BF16),
                pltpu.VMEM(rows, BF16),
                pltpu.VMEM((4, H, 128), F32), pltpu.VMEM((4, H, 128), F32), pltpu.VMEM((4, H, 1024), F32),
                pltpu.VMEM((4, 8, DH), F32), pltpu.VMEM((4, 8, WIN), F32), pltpu.VMEM((4, 8, DH), F32),
                pltpu.VMEM((4, 8, 8 * DH), F32), pltpu.VMEM((4, 8, 8 * DH), F32),
                pltpu.VMEM((1, 2 * DM), A_x.dtype), pltpu.SemaphoreType.DMA(()),
            ],
            compiler_params=pltpu.CompilerParams(vmem_limit_bytes=64 * 1024 * 1024),
        )(
            A_x.reshape(1, DM), A_k_cache.reshape(H, SK, DH), A_v_cache.reshape(H, SK, DH),
            A_wq.reshape(4, 128, H * DH), A_wo.reshape(rows),
            B_x.reshape(1, DM), B_c_kv.reshape(rows),
            B_w_q.reshape(slab), B_w_uk.reshape(slab), B_w_uv.reshape(slab), B_w_o.reshape(rows),
        )
        return out.reshape(1, 1, 2 * DM)
    return kernel


pallas_concat_heads__sliding_block_cached__compressed_kv_cla__decode_kernel = jax.jit(make())
```

```python
import functools

import jax
import jax.numpy as jnp
from jax import lax
import jax.experimental.pallas as pl
import jax.experimental.pallas.tpu as pltpu

F32 = jnp.float32
BF16 = jnp.bfloat16
H, DH = 32, 128
DM, DC = 512, 512
SK, WIN = 4096, 1024
NT = (((1,), (1,)), ((), ()))

V_START, OUT_START, END = 32, 64, 96
AHEAD = 10
LEAD = 24
A_CUTS = (0, 8, 16, 24, 28, 30)
B_CUTS = (0, 8, 16, 24, 32)
B_EARLY = 12
LAST_STREAMS = ((0, 3), (3, 4))


def _mul(i, n):
    return i * n if isinstance(i, int) else pl.multiple_of(i * n, n)


def _divmod(j, n):
    return divmod(j, n) if isinstance(j, int) else (lax.div(j, n), lax.rem(j, n))


def _interval(cuts, j):
    if isinstance(j, int):
        return sum(j >= c for c in cuts[1:-1])
    return sum((j >= c).astype(jnp.int32) for c in cuts[1:-1])


def _start(copies, lead=0):
    for n, c in enumerate(copies):
        c.start(priority=1 if n < lead else n % 2)


def _wait_filled(buf, sem):
    pltpu.make_async_copy(buf, buf, sem).wait()


def _slab_piece(src, dst, sem, u, j):
    i, s = _divmod(j, 8)
    idx = (u, i, pl.ds(_mul(s, 4), 4))
    return pltpu.make_async_copy(src.at[idx], dst.at[idx], sem)


def _row_piece(src, dst, sem, u, j):
    idx = (u, pl.ds(_mul(j, 32), 32))
    return pltpu.make_async_copy(src.at[idx], dst.at[idx], sem)


def _wide_piece(src, dst, sem, u, j):
    t, half = _divmod(j, 2)
    idx = (u, pl.ds(_mul(t, 8), 8), pl.ds(_mul(half, 2048), 2048))
    return pltpu.make_async_copy(src.at[idx], dst.at[idx], sem)


def _cache_round(src, dst, sem, j):
    t, g = _divmod(j, 4)
    r = _mul(t, 128)
    return [
        pltpu.make_async_copy(
            src.at[8 * g + u, pl.ds(SK - WIN + r, 128)], dst.at[8 * g + u, pl.ds(r, 128)], sem)
        for u in range(8)
    ]


def _flat_heads(o):
    return jnp.concatenate([jnp.broadcast_to(o[i:i + 1], (8, DH)) for i in range(8)], axis=1)


def _kernel(ax_h, k_h, v_h, wq_h, wo_h, bx_h, c_h, bwq_h, wuk_h, wuv_h, bwo_h, out_h,
            ax, k_v, v_v, wq_v, wo_v, bx, c_v, bwq_v, wuk_v, wuv_v, bwo_v,
            skew_s, qlat_s, sb_s, qa_s, pa_s, la_s, oa_s, ob_s, out_v, out_sem):
    put_out = pltpu.make_async_copy(out_v, out_h, out_sem)

    def project(a_sems, b_sems):
        def out_round(j):
            copies = []
            for u in range(4):
                if isinstance(j, int) and j >= A_CUTS[-1]:
                    a_sem = a_sems.at[len(A_CUTS) - 1 + (u >= LAST_STREAMS[1][0])]
                else:
                    a_sem = a_sems.at[_interval(A_CUTS, j)]
                copies.append(_row_piece(bwo_h, bwo_v, b_sems.at[_interval(B_CUTS, j)], u, j))
                copies.append(_row_piece(wo_h, wo_v, a_sem, u, j))
            return copies

        started = 0

        def start_round(sems, j, lo, hi):
            for a, b, copies in (
                    (0, V_START, lambda i: _cache_round(k_h, k_v, sems.at[5], i)),
                    (V_START, OUT_START, lambda i: _cache_round(v_h, v_v, sems.at[6], i)),
                    (OUT_START, END, out_round)):
                if a <= lo and hi < b:
                    _start(copies(j - a))
                elif lo < b and a <= hi:
                    pl.when((j >= a) & (j < b))(lambda: _start(copies(j - a)))

        def start_upto(sems, upto):
            nonlocal started
            lo, hi = started, min(upto, END)
            if lo >= hi:
                return
            if hi <= OUT_START:
                pl.loop(lo, hi)(lambda j: start_round(sems, j, lo, hi - 1))
            else:
                for j in range(lo, hi):
                    start_round(sems, j, j, j)
            started = hi

        def feeder(sems, per):
            nonlocal started
            base = started
            stop = OUT_START if base < OUT_START else OUT_START + A_CUTS[-1]
            started = min(base + 4 * per, stop)

            def feed(step, part, parts):
                for r in range(per):
                    lo, hi = base + r, base + 3 * per + r
                    if r * parts // per != part or lo >= stop:
                        continue
                    j = base + step * per + r
                    if hi < stop:
                        start_round(sems, j, lo, hi)
                    else:
                        pl.when(j < stop)(functools.partial(start_round, sems, j, lo, stop - 1))
            return feed

        def attend(sems):
            def weights_round(j):
                copies = []
                for u in range(4):
                    copies += [
                        _slab_piece(bwq_h, bwq_v, sems.at[0], u, j),
                        _slab_piece(wuk_h, wuk_v, sems.at[1], u, j),
                        _row_piece(c_h, c_v, sems.at[2], u, j),
                        _wide_piece(wq_h, wq_v, sems.at[3], u, j),
                        _slab_piece(wuv_h, wuv_v, sems.at[4], u, j),
                    ]
                return copies

            _start(weights_round(0) + weights_round(1), LEAD)
            get_ax = pltpu.make_async_copy(ax_h, ax, sems.at[7])
            get_bx = pltpu.make_async_copy(bx_h, bx, sems.at[8])
            get_ax.start()
            get_bx.start()
            pl.loop(2, 32)(lambda j: _start(weights_round(j)))
            start_upto(sems, AHEAD)

            row = lax.broadcasted_iota(jnp.int32, (H, 128), 0)
            lane = lax.broadcasted_iota(jnp.int32, (H, 128), 1)
            own_head = (lane & (H - 1)) == row
            row8 = lax.broadcasted_iota(jnp.int32, (8, DH), 0)

            def skew(v, sign):
                for bit in range(5):
                    moved = pltpu.roll(v, (sign * (1 << bit)) % 128, 1)
                    v = jnp.where(((row >> bit) & 1) == 1, moved, v)
                return v

            def contract_slabs(w_v, feed):
                def step(b, acc):
                    vs = skew_s[b]
                    for s in range(32):
                        feed(b, s, 32)
                        lhs = jnp.where(own_head, pltpu.roll(vs, 128 - s, 1) if s else vs, 0.0)
                        acc += jnp.dot(lhs.astype(BF16), w_v[b, :, s].reshape(128, DH),
                                       preferred_element_type=F32)
                    return acc
                return lax.fori_loop(0, 4, step, jnp.zeros((H, DH), F32))

            get_ax.wait()
            get_bx.wait()
            xa = ax[...].astype(F32)
            xb = bx[...].astype(F32)
            for b in range(4):
                skew_s[b] = skew(jnp.broadcast_to(xb[:, 128 * b:128 * (b + 1)], (H, 128)), 1)
                qa_s[b] = jnp.broadcast_to(xa[:, 128 * b:128 * (b + 1)], (8, 128))

            _wait_filled(bwq_v, sems.at[0])
            qb = contract_slabs(bwq_v, feeder(sems, 1)).astype(BF16)

            _wait_filled(wuk_v, sems.at[1])
            feed_qlat = feeder(sems, 4)

            @pl.loop(0, 4)
            def _(b):
                acc = jnp.zeros((H, 128), F32)
                for s in range(32):
                    feed_qlat(b, s, 32)
                    r = lax.dot_general(qb, wuk_v[b, :, s].reshape(128, DH), NT,
                                        preferred_element_type=F32)
                    r = jnp.where(own_head, r, 0.0)
                    acc += pltpu.roll(r, s, 1) if s else r
                qlat_s[b] = skew(acc, -1)

            qlat = jnp.concatenate([qlat_s[b] for b in range(4)], axis=1).astype(BF16)

            _wait_filled(c_v, sems.at[2])
            feed_scores = feeder(sems, 2)

            def score_step(j, m):
                for t in range(2):
                    feed_scores(j, t, 2)
                    s = lax.dot_general(qlat, c_v[j, 512 * t:512 * (t + 1)], NT,
                                        preferred_element_type=F32) * (DH ** -0.5)
                    sb_s[j, :, 512 * t:512 * (t + 1)] = s
                    for i in range(4):
                        m = jnp.maximum(m, s[:, 128 * i:128 * (i + 1)])
                return m

            m = lax.fori_loop(0, 4, score_step, jnp.full((H, 128), -jnp.inf, F32))
            m = jnp.max(m, axis=1, keepdims=True)
            feed_context = feeder(sems, 2)

            def context_step(j, carry):
                l, acc = carry
                for t in range(2):
                    feed_context(j, t, 2)
                    p = jnp.exp(sb_s[j, :, 512 * t:512 * (t + 1)] - m)
                    for i in range(4):
                        l += p[:, 128 * i:128 * (i + 1)]
                    acc += jnp.dot(p.astype(BF16), c_v[j, 512 * t:512 * (t + 1)],
                                   preferred_element_type=F32)
                return l, acc

            l, ctx_lat = lax.fori_loop(
                0, 4, context_step, (jnp.zeros((H, 128), F32), jnp.zeros((H, DC), F32)))
            ctx_lat = ctx_lat / jnp.sum(l, axis=1, keepdims=True)
            for b in range(4):
                skew_s[b] = skew(ctx_lat[:, 128 * b:128 * (b + 1)], 1)

            _wait_filled(wq_v, sems.at[3])
            feed_q = feeder(sems, 1)

            def q_step(j, acc):
                x8 = qa_s[j].astype(BF16)
                new = []
                for g in range(4):
                    feed_q(j, g, 4)
                    r = jnp.dot(x8, wq_v[j, :, 1024 * g:1024 * (g + 1)], preferred_element_type=F32)
                    a = acc[g]
                    for i in range(8):
                        a += jnp.where(row8 == i, r[:, DH * i:DH * (i + 1)], 0.0)
                    new.append(a)
                return tuple(new)

            qa = lax.fori_loop(0, 4, q_step, tuple(jnp.zeros((8, DH), F32) for _ in range(4)))
            for g in range(4):
                qa_s[g] = qa[g]

            _wait_filled(wuv_v, sems.at[4])
            ctx = contract_slabs(wuv_v, feeder(sems, 1))
            for g in range(4):
                ob_s[g] = _flat_heads(ctx[8 * g:8 * (g + 1)])

            start_upto(sems, V_START + AHEAD)
            _wait_filled(k_v, sems.at[5])
            feed_window = feeder(sems, 3)
            row8_win = lax.broadcasted_iota(jnp.int32, (8, WIN), 0)

            @pl.loop(0, 4)
            def _(g):
                q = qa_s[g].astype(BF16)
                s = jnp.zeros((8, WIN), F32)
                for i in range(8):
                    feed_window(g, i, 8)
                    r = lax.dot_general(q, k_v[8 * g + i], NT, preferred_element_type=F32)
                    s = jnp.where(row8_win == i, r, s)
                s = s * (DH ** -0.5)
                p = jnp.exp(s - jnp.max(s, axis=1, keepdims=True))
                pa_s[g] = p
                la_s[g] = jnp.broadcast_to(jnp.sum(p, axis=1, keepdims=True), (8, DH))

            start_upto(sems, OUT_START + AHEAD)
            _wait_filled(v_v, sems.at[6])
            feed_values = feeder(sems, 2)

            @pl.loop(0, 4)
            def _(g):
                p = pa_s[g].astype(BF16)
                o = jnp.zeros((8, DH), F32)
                for i in range(8):
                    feed_values(g, i, 8)
                    r = jnp.dot(p, v_v[8 * g + i], preferred_element_type=F32)
                    o = jnp.where(row8 == i, r, o)
                oa_s[g] = _flat_heads(o / la_s[g])

        pl.run_scoped(attend, pltpu.SemaphoreType.DMA((9,)))

        last = 32 * A_CUTS[-1]
        last_cols = [
            jnp.broadcast_to(oa_s[u, 0:1, 896:], (128, 128)).T[last - 896:] for u in range(4)]
        work = sorted([(B_CUTS[i + 1] - B_EARLY, 0, i) for i in range(len(B_CUTS) - 1)] +
                      [(A_CUTS[i + 1], 1, i) for i in range(len(A_CUTS) - 1)])
        acc = [jnp.zeros((8, DM), F32), jnp.zeros((8, DM), F32)]
        for _, side, i in work:
            o_s, w_v, sems, cuts = (
                (ob_s, bwo_v, b_sems, B_CUTS), (oa_s, wo_v, a_sems, A_CUTS))[side]
            r0, r1 = 32 * cuts[i], 32 * cuts[i + 1]
            start_upto(None, OUT_START + cuts[i + 1] + AHEAD)
            lhs = jnp.concatenate([o_s[u, :, r0:r1] for u in range(4)], axis=1).astype(BF16)
            _wait_filled(w_v.at[:, pl.ds(r0, r1 - r0)], sems.at[i])
            acc[side] += jnp.dot(lhs, w_v[:, r0:r1].reshape(4 * (r1 - r0), DM),
                                 preferred_element_type=F32)
            if side == 0 and i == len(B_CUTS) - 2:
                out_v[:, DM:] = acc[0][0:1].astype(out_v.dtype)

        part = jnp.zeros((8, DM), F32)
        for i, (u0, u1) in enumerate(LAST_STREAMS):
            _wait_filled(wo_v.at[pl.ds(u0, u1 - u0), pl.ds(last, 1024 - last)],
                         a_sems.at[len(A_CUTS) - 1 + i])
            for u in range(u0, u1):
                w = wo_v[u, last:].astype(F32)
                for r in range(0, 1024 - last, 8):
                    part += w[r:r + 8] * jnp.concatenate([last_cols[u][r:r + 8]] * 4, axis=1)
        out_v[:, :DM] = (acc[1][0:1] + jnp.sum(part, axis=0, keepdims=True)).astype(out_v.dtype)
        assert started == END
        put_out.start()

    pl.run_scoped(project,
                  pltpu.SemaphoreType.DMA((len(A_CUTS) - 1 + len(LAST_STREAMS),)),
                  pltpu.SemaphoreType.DMA((len(B_CUTS) - 1,)))
    put_out.wait()


@jax.jit
def pallas_concat_heads__sliding_block_cached__compressed_kv_cla__decode_kernel(
    A_x: jax.Array,
    A_k_cache: jax.Array,
    A_v_cache: jax.Array,
    A_wq: jax.Array,
    A_wo: jax.Array,
    B_x: jax.Array,
    B_c_kv: jax.Array,
    B_w_q: jax.Array,
    B_w_uk: jax.Array,
    B_w_uv: jax.Array,
    B_w_o: jax.Array,
):
    cache, wide, rows, slabs = (H, SK, DH), (4, 128, H * DH), (4, 1024, DM), (4, 4, 32, H, DH)
    hbm = pl.BlockSpec(memory_space=pltpu.MemorySpace.HBM)
    out = pl.pallas_call(
        _kernel,
        in_specs=[hbm] * 11,
        out_specs=hbm,
        out_shape=jax.ShapeDtypeStruct((1, 2 * DM), A_x.dtype),
        scratch_shapes=[
            pltpu.VMEM((1, DM), BF16),
            pltpu.VMEM((H, WIN, DH), BF16),
            pltpu.VMEM((H, WIN, DH), BF16),
            pltpu.VMEM(wide, BF16),
            pltpu.VMEM(rows, BF16),
            pltpu.VMEM((1, DM), BF16),
            pltpu.VMEM(rows, BF16),
            pltpu.VMEM(slabs, BF16),
            pltpu.VMEM(slabs, BF16),
            pltpu.VMEM(slabs, BF16),
            pltpu.VMEM(rows, BF16),
            pltpu.VMEM((4, H, 128), F32),
            pltpu.VMEM((4, H, 128), F32),
            pltpu.VMEM((4, H, 1024), F32),
            pltpu.VMEM((4, 8, DH), F32),
            pltpu.VMEM((4, 8, WIN), F32),
            pltpu.VMEM((4, 8, DH), F32),
            pltpu.VMEM((4, 8, 8 * DH), F32),
            pltpu.VMEM((4, 8, 8 * DH), F32),
            pltpu.VMEM((1, 2 * DM), A_x.dtype),
            pltpu.SemaphoreType.DMA(()),
        ],
        compiler_params=pltpu.CompilerParams(vmem_limit_bytes=64 * 1024 * 1024),
    )(
        A_x.reshape(1, DM), A_k_cache.reshape(cache), A_v_cache.reshape(cache),
        A_wq.reshape(wide), A_wo.reshape(rows),
        B_x.reshape(1, DM), B_c_kv.reshape(rows),
        B_w_q.reshape(slabs), B_w_uk.reshape(slabs), B_w_uv.reshape(slabs), B_w_o.reshape(rows),
    )
    return out.reshape(1, 1, 2 * DM)
```

```python
import functools

import jax
import jax.numpy as jnp
from jax import lax
import jax.experimental.pallas as pl
import jax.experimental.pallas.tpu as pltpu

F32 = jnp.float32
BF16 = jnp.bfloat16
H, DH = 32, 128
DM, DC = 512, 512
SK, WIN = 4096, 1024
NT = (((1,), (1,)), ((), ()))

V_START, OUT_START, END = 32, 64, 96
AHEAD = 11
LEAD = 28
A_CUTS = (0, 8, 16, 24, 28, 30)
B_CUTS = (0, 8, 16, 24, 32)
B_EARLY = 12
A_LAST = ((30, 0, 4), (31, 0, 3), (31, 3, 4))


def _mul(i, n):
    return i * n if isinstance(i, int) else pl.multiple_of(i * n, n)


def _divmod(j, n):
    return divmod(j, n) if isinstance(j, int) else (lax.div(j, n), lax.rem(j, n))


def _interval(cuts, j):
    if isinstance(j, int):
        return sum(j >= c for c in cuts[1:-1])
    return sum((j >= c).astype(jnp.int32) for c in cuts[1:-1])


def _start(copies, lead=0):
    for n, c in enumerate(copies):
        c.start(priority=1 if n < lead else n % 2)


def _wait_filled(buf, sem):
    pltpu.make_async_copy(buf, buf, sem).wait()


def _slab_piece(src, dst, sem, u, j):
    i, s = _divmod(j, 8)
    idx = (u, i, pl.ds(_mul(s, 4), 4))
    return pltpu.make_async_copy(src.at[idx], dst.at[idx], sem)


def _row_piece(src, dst, sem, u, j):
    idx = (u, pl.ds(_mul(j, 32), 32))
    return pltpu.make_async_copy(src.at[idx], dst.at[idx], sem)


def _wide_piece(src, dst, sem, u, j):
    t, half = _divmod(j, 2)
    idx = (u, pl.ds(_mul(t, 8), 8), pl.ds(_mul(half, 2048), 2048))
    return pltpu.make_async_copy(src.at[idx], dst.at[idx], sem)


def _cache_round(src, dst, sem, j):
    t, g = _divmod(j, 4)
    r = _mul(t, 128)
    heads = [8 * (u % 4) + 2 * g + u // 4 for u in range(8)]
    return [
        pltpu.make_async_copy(
            src.at[h, pl.ds(SK - WIN + r, 128)], dst.at[h, pl.ds(r, 128)], sem)
        for h in heads
    ]


def _flat_heads(o):
    return jnp.concatenate([jnp.broadcast_to(o[i:i + 1], (8, DH)) for i in range(8)], axis=1)


def _kernel(ax_h, k_h, v_h, wq_h, wo_h, bx_h, c_h, bwq_h, wuk_h, wuv_h, bwo_h, out_h,
            ax, k_v, v_v, wq_v, wo_v, bx, c_v, bwq_v, wuk_v, wuv_v, bwo_v,
            skew_s, qlat_s, sb_s, qa_s, pa_s, la_s, oa_s, ob_s, out_v, out_sem):
    put_out = pltpu.make_async_copy(out_v, out_h, out_sem)

    def project(a_sems, b_sems):
        def out_round(j):
            p, half = _divmod(j, 2)
            copies = []
            for u in range(4):
                if isinstance(j, int) and j >= A_CUTS[-1]:
                    group = [r == j and u0 <= u < u1 for r, u0, u1 in A_LAST].index(True)
                    a_sem = a_sems.at[len(A_CUTS) - 1 + group]
                else:
                    a_sem = a_sems.at[_interval(A_CUTS, j)]
                b_sem = b_sems.at[_interval(B_CUTS, j)]
                idx = (u, half, pl.ds(_mul(p, 32), 32))
                copies.append(pltpu.make_async_copy(bwo_h.at[idx], bwo_v.at[idx], b_sem))
                copies.append(pltpu.make_async_copy(wo_h.at[idx], wo_v.at[idx], a_sem))
            return copies

        started = 0

        def start_round(sems, j, lo, hi):
            for a, b, copies in (
                    (0, V_START, lambda i: _cache_round(k_h, k_v, sems.at[5], i)),
                    (V_START, OUT_START, lambda i: _cache_round(v_h, v_v, sems.at[6], i)),
                    (OUT_START, END, out_round)):
                if a <= lo and hi < b:
                    _start(copies(j - a))
                elif lo < b and a <= hi:
                    pl.when((j >= a) & (j < b))(lambda: _start(copies(j - a)))

        def start_upto(sems, upto):
            nonlocal started
            lo, hi = started, min(upto, END)
            if lo >= hi:
                return
            if hi <= OUT_START:
                pl.loop(lo, hi)(lambda j: start_round(sems, j, lo, hi - 1))
            else:
                for j in range(lo, hi):
                    start_round(sems, j, j, j)
            started = hi

        def feeder(sems, per):
            nonlocal started
            base = started
            stop = OUT_START if base < OUT_START else OUT_START + A_CUTS[-1]
            started = min(base + 4 * per, stop)

            def feed(step, part, parts):
                for r in range(per):
                    lo, hi = base + r, base + 3 * per + r
                    if r * parts // per != part or lo >= stop:
                        continue
                    j = base + step * per + r
                    if hi < stop:
                        start_round(sems, j, lo, hi)
                    else:
                        pl.when(j < stop)(functools.partial(start_round, sems, j, lo, stop - 1))
            return feed

        def attend(sems):
            def weights_round(j):
                copies = []
                for u in range(4):
                    copies += [
                        _wide_piece(wq_h, wq_v, sems.at[3], u, j),
                        _slab_piece(bwq_h, bwq_v, sems.at[0], u, j),
                        _slab_piece(wuk_h, wuk_v, sems.at[1], u, j),
                        _slab_piece(wuv_h, wuv_v, sems.at[4], u, j),
                        _row_piece(c_h, c_v, sems.at[2], u, j),
                    ]
                return copies

            _start(weights_round(0) + weights_round(1), LEAD)
            get_ax = pltpu.make_async_copy(ax_h, ax, sems.at[7])
            get_bx = pltpu.make_async_copy(bx_h, bx, sems.at[8])
            get_ax.start()
            get_bx.start()
            pl.loop(2, 32)(lambda j: _start(weights_round(j)))
            start_upto(sems, AHEAD)

            row = lax.broadcasted_iota(jnp.int32, (H, 128), 0)
            lane = lax.broadcasted_iota(jnp.int32, (H, 128), 1)
            own_head = (lane & (H - 1)) == row
            row8 = lax.broadcasted_iota(jnp.int32, (8, DH), 0)

            def skew(v, sign):
                for bit in range(5):
                    moved = pltpu.roll(v, (sign * (1 << bit)) % 128, 1)
                    v = jnp.where(((row >> bit) & 1) == 1, moved, v)
                return v

            def contract_slabs(w_v, feed):
                def step(b, acc):
                    vs = skew_s[b]
                    for s in range(32):
                        feed(b, s, 32)
                        lhs = jnp.where(own_head, pltpu.roll(vs, 128 - s, 1) if s else vs, 0.0)
                        acc += jnp.dot(lhs.astype(BF16), w_v[b, :, s].reshape(128, DH),
                                       preferred_element_type=F32)
                    return acc
                return lax.fori_loop(0, 4, step, jnp.zeros((H, DH), F32))

            get_ax.wait()
            get_bx.wait()
            xa = ax[...].astype(F32)
            xb = bx[...].astype(F32)
            for b in range(4):
                skew_s[b] = skew(jnp.broadcast_to(xb[:, 128 * b:128 * (b + 1)], (H, 128)), 1)
                qa_s[b] = jnp.broadcast_to(xa[:, 128 * b:128 * (b + 1)], (8, 128))

            _wait_filled(bwq_v, sems.at[0])
            qb = contract_slabs(bwq_v, feeder(sems, 1)).astype(BF16)

            _wait_filled(wuk_v, sems.at[1])
            feed_qlat = feeder(sems, 4)

            @pl.loop(0, 4)
            def _(b):
                acc = jnp.zeros((H, 128), F32)
                for s in range(32):
                    feed_qlat(b, s, 32)
                    r = lax.dot_general(qb, wuk_v[b, :, s].reshape(128, DH), NT,
                                        preferred_element_type=F32)
                    r = jnp.where(own_head, r, 0.0)
                    acc += pltpu.roll(r, s, 1) if s else r
                qlat_s[b] = skew(acc, -1)

            qlat = jnp.concatenate([qlat_s[b] for b in range(4)], axis=1).astype(BF16)

            _wait_filled(c_v, sems.at[2])
            feed_scores = feeder(sems, 2)

            def score_step(j, m):
                for t in range(2):
                    feed_scores(j, t, 2)
                    s = lax.dot_general(qlat, c_v[j, 512 * t:512 * (t + 1)], NT,
                                        preferred_element_type=F32) * (DH ** -0.5)
                    sb_s[j, :, 512 * t:512 * (t + 1)] = s
                    for i in range(4):
                        m = jnp.maximum(m, s[:, 128 * i:128 * (i + 1)])
                return m

            m = lax.fori_loop(0, 4, score_step, jnp.full((H, 128), -jnp.inf, F32))
            m = jnp.max(m, axis=1, keepdims=True)
            feed_context = feeder(sems, 2)

            def context_step(j, carry):
                l, acc = carry
                for t in range(2):
                    feed_context(j, t, 2)
                    p = jnp.exp(sb_s[j, :, 512 * t:512 * (t + 1)] - m)
                    for i in range(4):
                        l += p[:, 128 * i:128 * (i + 1)]
                    acc += jnp.dot(p.astype(BF16), c_v[j, 512 * t:512 * (t + 1)],
                                   preferred_element_type=F32)
                return l, acc

            l, ctx_lat = lax.fori_loop(
                0, 4, context_step, (jnp.zeros((H, 128), F32), jnp.zeros((H, DC), F32)))
            ctx_lat = ctx_lat / jnp.sum(l, axis=1, keepdims=True)
            for b in range(4):
                skew_s[b] = skew(ctx_lat[:, 128 * b:128 * (b + 1)], 1)

            _wait_filled(wq_v, sems.at[3])
            feed_q = feeder(sems, 1)

            def q_step(j, acc):
                x8 = qa_s[j].astype(BF16)
                new = []
                for g in range(4):
                    feed_q(j, g, 4)
                    r = jnp.dot(x8, wq_v[j, :, 1024 * g:1024 * (g + 1)], preferred_element_type=F32)
                    a = acc[g]
                    for i in range(8):
                        a += jnp.where(row8 == i, r[:, DH * i:DH * (i + 1)], 0.0)
                    new.append(a)
                return tuple(new)

            qa = lax.fori_loop(0, 4, q_step, tuple(jnp.zeros((8, DH), F32) for _ in range(4)))
            for g in range(4):
                qa_s[g] = qa[g]

            _wait_filled(wuv_v, sems.at[4])
            ctx = contract_slabs(wuv_v, feeder(sems, 1))
            for g in range(4):
                ob_s[g] = _flat_heads(ctx[8 * g:8 * (g + 1)])

            start_upto(sems, V_START + AHEAD)
            _wait_filled(k_v, sems.at[5])
            feed_window = feeder(sems, 3)
            row8_win = lax.broadcasted_iota(jnp.int32, (8, WIN), 0)

            @pl.loop(0, 4)
            def _(g):
                q = qa_s[g].astype(BF16)
                s = jnp.zeros((8, WIN), F32)
                for i in range(8):
                    feed_window(g, i, 8)
                    r = lax.dot_general(q, k_v[8 * g + i], NT, preferred_element_type=F32)
                    s = jnp.where(row8_win == i, r, s)
                s = s * (DH ** -0.5)
                p = jnp.exp(s - jnp.max(s, axis=1, keepdims=True))
                pa_s[g] = p
                la_s[g] = jnp.broadcast_to(jnp.sum(p, axis=1, keepdims=True), (8, DH))

            start_upto(sems, OUT_START + AHEAD)
            _wait_filled(v_v, sems.at[6])
            feed_values = feeder(sems, 2)

            @pl.loop(0, 4)
            def _(g):
                p = pa_s[g].astype(BF16)
                o = jnp.zeros((8, DH), F32)
                for i in range(8):
                    feed_values(g, i, 8)
                    r = jnp.dot(p, v_v[8 * g + i], preferred_element_type=F32)
                    o = jnp.where(row8 == i, r, o)
                oa_s[g] = _flat_heads(o / la_s[g])

        pl.run_scoped(attend, pltpu.SemaphoreType.DMA((9,)))

        last_cols = [
            [jnp.broadcast_to(oa_s[u, 0:1, end - 128:end], (128, 128)).T[96:] for end in (512, 1024)]
            for u in range(4)]
        work = sorted([(B_CUTS[i + 1] - B_EARLY, 0, i) for i in range(len(B_CUTS) - 1)] +
                      [(A_CUTS[i + 1], 1, i) for i in range(len(A_CUTS) - 1)])
        acc = [jnp.zeros((8, DM), F32), jnp.zeros((8, DM), F32)]
        for _, side, i in work:
            o_s, w_v, sems, cuts = (
                (ob_s, bwo_v, b_sems, B_CUTS), (oa_s, wo_v, a_sems, A_CUTS))[side]
            r0, r1 = 16 * cuts[i], 16 * cuts[i + 1]
            start_upto(None, OUT_START + cuts[i + 1] + AHEAD)
            lhs = jnp.concatenate(
                [o_s[u, :, c + r0:c + r1] for u in range(4) for c in (0, 512)], axis=1)
            _wait_filled(w_v.at[:, :, pl.ds(r0, r1 - r0)], sems.at[i])
            acc[side] += jnp.dot(lhs.astype(BF16), w_v[:, :, r0:r1].reshape(8 * (r1 - r0), DM),
                                 preferred_element_type=F32)
            if side == 0 and i == len(B_CUTS) - 2:
                out_v[:, DM:] = acc[0][0:1].astype(out_v.dtype)

        part = jnp.zeros((8, DM), F32)
        for group, (j, u0, u1) in enumerate(A_LAST):
            half, r0 = j % 2, 32 * (j // 2)
            _wait_filled(wo_v.at[pl.ds(u0, u1 - u0), half, pl.ds(r0, 32)],
                         a_sems.at[len(A_CUTS) - 1 + group])
            for u in range(u0, u1):
                w = wo_v[u, half, r0:r0 + 32].astype(F32)
                for r in range(0, 32, 8):
                    col = last_cols[u][half][r:r + 8]
                    part += w[r:r + 8] * jnp.concatenate([col] * 4, axis=1)
        out_v[:, :DM] = (acc[1][0:1] + jnp.sum(part, axis=0, keepdims=True)).astype(out_v.dtype)
        assert started == END
        put_out.start()

    pl.run_scoped(project,
                  pltpu.SemaphoreType.DMA((len(A_CUTS) - 1 + len(A_LAST),)),
                  pltpu.SemaphoreType.DMA((len(B_CUTS) - 1,)))
    put_out.wait()


@jax.jit
def pallas_concat_heads__sliding_block_cached__compressed_kv_cla__decode_kernel(
    A_x: jax.Array,
    A_k_cache: jax.Array,
    A_v_cache: jax.Array,
    A_wq: jax.Array,
    A_wo: jax.Array,
    B_x: jax.Array,
    B_c_kv: jax.Array,
    B_w_q: jax.Array,
    B_w_uk: jax.Array,
    B_w_uv: jax.Array,
    B_w_o: jax.Array,
):
    cache, wide, rows = (H, SK, DH), (4, 128, H * DH), (4, 1024, DC)
    slabs, proj = (4, 4, 32, H, DH), (4, 2, 512, DM)
    hbm = pl.BlockSpec(memory_space=pltpu.MemorySpace.HBM)
    out = pl.pallas_call(
        _kernel,
        in_specs=[hbm] * 11,
        out_specs=hbm,
        out_shape=jax.ShapeDtypeStruct((1, 2 * DM), A_x.dtype),
        scratch_shapes=[
            pltpu.VMEM((1, DM), BF16),
            pltpu.VMEM((H, WIN, DH), BF16),
            pltpu.VMEM((H, WIN, DH), BF16),
            pltpu.VMEM(wide, BF16),
            pltpu.VMEM(proj, BF16),
            pltpu.VMEM((1, DM), BF16),
            pltpu.VMEM(rows, BF16),
            pltpu.VMEM(slabs, BF16),
            pltpu.VMEM(slabs, BF16),
            pltpu.VMEM(slabs, BF16),
            pltpu.VMEM(proj, BF16),
            pltpu.VMEM((4, H, 128), F32),
            pltpu.VMEM((4, H, 128), F32),
            pltpu.VMEM((4, H, 1024), F32),
            pltpu.VMEM((4, 8, DH), F32),
            pltpu.VMEM((4, 8, WIN), F32),
            pltpu.VMEM((4, 8, DH), F32),
            pltpu.VMEM((4, 8, 8 * DH), F32),
            pltpu.VMEM((4, 8, 8 * DH), F32),
            pltpu.VMEM((1, 2 * DM), A_x.dtype),
            pltpu.SemaphoreType.DMA(()),
        ],
        compiler_params=pltpu.CompilerParams(vmem_limit_bytes=64 * 1024 * 1024),
    )(
        A_x.reshape(1, DM), A_k_cache.reshape(cache), A_v_cache.reshape(cache),
        A_wq.reshape(wide), A_wo.reshape(proj),
        B_x.reshape(1, DM), B_c_kv.reshape(rows),
        B_w_q.reshape(slabs), B_w_uk.reshape(slabs), B_w_uv.reshape(slabs), B_w_o.reshape(proj),
    )
    return out.reshape(1, 1, 2 * DM)
```
